```python
import jax
import jax.numpy as jnp

def _softmax(x, axis=-1):
    return jax.nn.softmax(x, axis=axis)
def _gelu(x):
    return jax.nn.gelu(x, approximate=True)
def _silu(x):
    return jax.nn.silu(x)
def _sigmoid(x):
    return jax.nn.sigmoid(x)
def _layernorm(x, axis=-1, eps=1e-5):
    m = jnp.mean(x, axis=axis, keepdims=True)
    v = jnp.var(x, axis=axis, keepdims=True)
    return (x - m) / jnp.sqrt(v + eps)
def _scatter_add(tgt, idx, src, axis=0):
    return tgt.at[idx].add(src)
def _segment_sum(src, seg, n):
    return jax.ops.segment_sum(src, seg, n)
class _Rng:
    def __init__(self, key):
        self._k = key
    def _next(self):
        self._k, sub = jax.random.split(self._k)
        return sub
    def normal(self, shape):
        return jax.random.normal(self._next(), shape, dtype=jnp.bfloat16)
    def randint(self, lo, hi, shape):
        return jax.random.randint(self._next(), shape, lo, hi, dtype=jnp.int32)
    def uniform(self, shape, lo=0.0, hi=1.0):
        return jax.random.uniform(self._next(), shape, jnp.bfloat16, lo, hi)
    def permutation(self, n):
        return jax.random.permutation(self._next(), n)


kernel_name = 'parallel_sum__compressed_kv_cla__geglu_ffn__decode'

def _fwd_setup_inputs():
    _rng = _Rng(jax.random.key(int.from_bytes(__import__("os").urandom(4), "little")))
    _w = (lambda a: (lambda t: t.astype(jnp.bfloat16) if jnp.issubdtype(t.dtype, jnp.floating) else t)(jnp.asarray(a)))
    def _A_setup():
        B, H, Sq, Sk, D, M = 8, 32, 1, 4096, 128, 512
        Dc = 4 * D
        return {
            "x": _w((lambda *s: _rng.normal(s) * 0.05)(B, Sq, M)),
            "c_kv": _w((lambda *s: _rng.normal(s) * 0.05)(B, Sk, Dc)),
            "w_q": _w((lambda *s: _rng.normal(s) * 0.05)(M, H, D) * (M ** -0.5)),
            "w_uk": _w((lambda *s: _rng.normal(s) * 0.05)(Dc, H, D) * (Dc ** -0.5)),
            "w_uv": _w((lambda *s: _rng.normal(s) * 0.05)(Dc, H, D) * (Dc ** -0.5)),
            "w_o": _w((lambda *s: _rng.normal(s) * 0.05)(H, D, M) * ((H * D) ** -0.5)),
        }
    _A_in = _A_setup()

    def _B_setup():
        B, S, D, F = 8, 1, 512, 1376
        return {
            "x": _w((lambda *s: _rng.normal(s) * 0.05)(B, S, D)),
            "w_gate": _w((lambda *s: _rng.normal(s) * 0.05)(D, F)),
            "w_up": _w((lambda *s: _rng.normal(s) * 0.05)(D, F)),
            "w_down": _w((lambda *s: _rng.normal(s) * 0.05)(F, D)),
        }
    _B_in = _B_setup()

    return {
        "A_x": _A_in["x"],
        "A_c_kv": _A_in["c_kv"],
        "A_w_q": _A_in["w_q"],
        "A_w_uk": _A_in["w_uk"],
        "A_w_uv": _A_in["w_uv"],
        "A_w_o": _A_in["w_o"],
        "B_x": _B_in["x"],
        "B_w_gate": _B_in["w_gate"],
        "B_w_up": _B_in["w_up"],
        "B_w_down": _B_in["w_down"],
    }

def _fwd_reference(A_x, A_c_kv, A_w_q, A_w_uk, A_w_uv, A_w_o, B_x, B_w_gate, B_w_up, B_w_down):
    def _A_ref(x, c_kv, w_q, w_uk, w_uv, w_o):
        B, Sq, M = x.shape[0], x.shape[1], x.shape[2]
        Sk = c_kv.shape[1]
        H, D = w_q.shape[1], w_q.shape[2]
        q = jnp.einsum("bqm,mhd->bhqd", x, w_q)
        k = jnp.einsum("bkc,chd->bhkd", c_kv, w_uk)
        v = jnp.einsum("bkc,chd->bhkd", c_kv, w_uv)
        scores = jnp.einsum("bhqd,bhkd->bhqk", q, k) * (D ** -0.5)
        off = Sk - Sq
        qi = jnp.arange(Sq)[:, None]
        kj = jnp.arange(Sk)[None, :]
        cmask = kj <= (qi + off)
        scores = jnp.where(cmask[None, None], scores, -1e9)
        p = _softmax(scores, axis=-1)
        ctx = jnp.einsum("bhqk,bhkd->bhqd", p, v)
        return jnp.einsum("bhqd,hdm->bqm", ctx, w_o)

    def _B_ref(x, w_gate, w_up, w_down):
        return (_gelu(x @ w_gate) * (x @ w_up)) @ w_down

    x = A_x
    xn = _layernorm(x, axis=-1)
    return x + _A_ref(xn, A_c_kv, A_w_q, A_w_uk, A_w_uv, A_w_o) + _B_ref(xn, B_w_gate, B_w_up, B_w_down)


def setup_inputs():
    _inp = _fwd_setup_inputs()
    _gk = jax.random.fold_in(jax.random.key(int.from_bytes(__import__("os").urandom(4), "little")), 2**31 - 1)
    _shapes = [[8, 1, 512]]
    _dtypes = ['bfloat16']
    _gks = jax.random.split(_gk, len(_shapes))
    _gs = [jax.random.normal(k, s, dtype=jnp.dtype(d)) * 0.05 for k, s, d in zip(_gks, _shapes, _dtypes)]
    _inp["grad_out"] = _gs[0]
    return _inp

def reference(A_x, A_c_kv, A_w_q, A_w_uk, A_w_uv, A_w_o, B_w_gate, B_w_up, B_w_down, B_x, grad_out):
    _const = dict(B_x=B_x)
    def _f(*_d):
        return _fwd_reference(**{'A_x': _d[0], 'A_c_kv': _d[1], 'A_w_q': _d[2], 'A_w_uk': _d[3], 'A_w_uv': _d[4], 'A_w_o': _d[5], 'B_w_gate': _d[6], 'B_w_up': _d[7], 'B_w_down': _d[8], **_const})
    _out, _vjp = jax.vjp(_f, A_x, A_c_kv, A_w_q, A_w_uk, A_w_uv, A_w_o, B_w_gate, B_w_up, B_w_down)
    _grads = _vjp(grad_out)
    _out0 = jnp.asarray(_out)
    return (_out0, *[jnp.asarray(_g) for _g in _grads])
```

```python
import jax
import jax.numpy as jnp
from jax.experimental import pallas as pl
from jax.experimental.pallas import tpu as pltpu

BF = jnp.bfloat16
F32 = jnp.float32

NN = (((1,), (0,)), ((), ()))
NT = (((1,), (1,)), ((), ()))
TN = (((0,), (0,)), ((), ()))
BNN = (((2,), (1,)), ((0,), (0,)))
BNT = (((2,), (2,)), ((0,), (0,)))
BTN = (((1,), (1,)), ((0,), (0,)))

LN_EPS = 1e-5
GELU_K0 = 0.7978845608028654
GELU_K1 = 0.044715

RUN_BYTES = 32 * 1024
N_STRIPS = 32
FFN_ROWS = 64
SWITCH = 5
TAIL_STRIPS = 16
VMEM_LIMIT = 110 * 1024 * 1024


def _dot(a, b, dims):
    return jax.lax.dot_general(a, b, dims, preferred_element_type=F32)


def _make_kernel(B, SK, CD, M, H, D, F):
    scale = float(D) ** -0.5
    lanes = 128
    hh = lanes // B
    assert hh * B == lanes and H % hh == 0 and D == lanes
    assert 0 < SWITCH < B - 1

    def kernel(x_hbm, c_hbm, wq_hbm, wuk_hbm, wuv_hbm, wo_hbm, wg_hbm, wu_hbm, wd_hbm, g_hbm,
               o_hbm, dx_hbm, dc_hbm, dwq_hbm, dwuk_hbm, dwuv_hbm, dwo_hbm, dwg_hbm, dwu_hbm, dwd_hbm,
               xs, gs, os_, dxs, cbuf, wq_r, wuk_r, wuv_r, wo, wq3, wuk3, wuv3, wg, wu, wd,
               a_all, r_all, xt_ref, rsem, wsem):
        reads = [(x_hbm, xs), (g_hbm, gs), (wg_hbm, wg), (wu_hbm, wu), (wd_hbm, wd),
                 (wq_hbm, wq_r), (wuk_hbm, wuk_r), (wo_hbm, wo), (wuv_hbm, wuv_r)]
        n_rd = len(reads)
        n_g = cbuf.shape[1]
        keep = N_STRIPS - TAIL_STRIPS

        def rd(i):
            src, dst = reads[i]
            return pltpu.make_async_copy(src, dst, rsem.at[i])

        def rd_c(b):
            return pltpu.make_async_copy(c_hbm.at[b], cbuf.at[b], rsem.at[n_rd + b])

        def rd_last(part):
            idx = [(pl.ds(0, n_g - 1),),
                   (n_g - 1, pl.ds(0, keep)),
                   (n_g - 1, pl.ds(keep, TAIL_STRIPS))][part]
            return pltpu.make_async_copy(c_hbm.at[(B - 1,) + idx], cbuf.at[(B - 1,) + idx],
                                         rsem.at[n_rd + B - 1 + part])

        for i in range(n_rd):
            rd(i).start()
        for b in range(B - 1):
            rd_c(b).start()
        for part in range(3):
            rd_last(part).start()

        def wr_c(b0, nb, sem):
            return [lambda j=j: pltpu.make_async_copy(cbuf.at[pl.ds(b0, nb), :, j],
                                                      dc_hbm.at[pl.ds(b0, nb), :, j], wsem.at[sem])
                    for j in range(N_STRIPS)]

        def wr_w(src, dst, sem):
            return [lambda j=j: pltpu.make_async_copy(src.at[:, j], dst.at[:, j], wsem.at[sem])
                    for j in range(N_STRIPS)]

        ffn_writes = []
        for r0 in range(0, F, FFN_ROWS):
            rows = pl.ds(r0, min(FFN_ROWS, F - r0))
            for sem, (src, dst) in enumerate([(wg, dwg_hbm), (wu, dwu_hbm), (wd, dwd_hbm)]):
                ffn_writes.append(lambda src=src, dst=dst, rows=rows, sem=sem:
                                  pltpu.make_async_copy(src.at[rows], dst.at[rows], wsem.at[sem]))
        SEM_SMALL, SEM_C, SEM_W = 3, 5, 7

        started = []

        def issue(copies, extra=()):
            done = 0
            for i, make in enumerate(copies):
                make().start()
                upto = (i + 1) * len(extra) // len(copies)
                for e in extra[done:upto]:
                    e().start()
                done = upto
            started.extend(copies)
            started.extend(extra)

        rd(0).wait()
        rd(1).wait()
        x = xs[...].astype(F32)
        g_b = gs[...]
        g = g_b.astype(F32)
        xc = x - jnp.mean(x, axis=-1, keepdims=True)
        rstd = jax.lax.rsqrt(jnp.mean(xc * xc, axis=-1, keepdims=True) + LN_EPS)
        xn = xc * rstd
        xn_b = xn.astype(BF)

        rd(2).wait()
        rd(3).wait()
        gate = _dot(xn_b, wg[...], NT)
        up = _dot(xn_b, wu[...], NT)
        th = jnp.tanh(GELU_K0 * (gate + GELU_K1 * gate * gate * gate))
        gl = 0.5 * gate * (1.0 + th)
        dgl = (0.5 * (1.0 + th)
               + 0.5 * gate * (1.0 - th * th) * GELU_K0 * (1.0 + 3.0 * GELU_K1 * gate * gate))
        hid_b = (gl * up).astype(BF)
        rd(4).wait()
        out_ffn = _dot(hid_b, wd[...], NN)
        dh = _dot(g_b, wd[...], NT)
        dgate_b = (dh * up * dgl).astype(BF)
        dup_b = (dh * gl).astype(BF)
        dxn_ffn = _dot(dgate_b, wg[...], NN) + _dot(dup_b, wu[...], NN)
        wg[...] = _dot(dgate_b, xn_b, TN).astype(BF)
        wu[...] = _dot(dup_b, xn_b, TN).astype(BF)
        wd[...] = _dot(hid_b, g_b, TN).astype(BF)

        def head_major(src, dst):
            rows = src.shape[1] * src.shape[2]

            def body(k, carry):
                r0 = pl.multiple_of(k * rows, rows)
                dst[:, pl.ds(r0, rows), :] = jnp.swapaxes(src[k].reshape(rows, H, D), 0, 1)
                return carry
            jax.lax.fori_loop(0, src.shape[0], body, 0)

        rd(5).wait()
        head_major(wq_r, wq3)
        q_b = _dot(jnp.broadcast_to(xn_b[None], (H, B, M)), wq3[...], BNN).astype(BF)
        rd(6).wait()
        head_major(wuk_r, wuk3)
        q_abs = _dot(q_b, wuk3[...], BNT) * scale
        rd(7).wait()
        g_bb = jnp.broadcast_to(g_b[None], (H, B, M))
        dctx_b = _dot(g_bb, wo[...].reshape(H, D, M), BNT).astype(BF)
        rd(8).wait()
        head_major(wuv_r, wuv3)
        dctx_abs = _dot(dctx_b, wuv3[...], BNT)
        a_all[...] = jnp.swapaxes(jnp.concatenate([q_abs, dctx_abs], axis=0), 0, 1).astype(BF)

        def batch(b, carry):
            @pl.when(b < B - 1)
            def _():
                rd_c(b).wait()

            @pl.when(b == B - 1)
            def _():
                rd_last(0).wait()
                rd_last(2).wait()

            @pl.when(b == SWITCH)
            def _():
                rd_last(1).wait()
                for make in wr_c(0, SWITCH, SEM_C):
                    make().start()

            a = a_all[b]
            s_all = _dot(a, cbuf[b].reshape(SK, CD), NT)
            s, dp = s_all[:H], s_all[H:]
            e = jnp.exp(s - jnp.max(s, axis=-1, keepdims=True))
            p = e * (1.0 / jnp.sum(e, axis=-1, keepdims=True))
            ds = p * (dp - jnp.sum(p * dp, axis=-1, keepdims=True))
            pm = jnp.concatenate([ds.astype(BF), p.astype(BF)], axis=0)
            r_all[b] = _dot(pm, cbuf[b].reshape(SK, CD), NN)
            cbuf[b] = _dot(pm, a, TN).astype(BF).reshape(cbuf.shape[1:])
            return carry

        jax.lax.fori_loop(0, B, batch, 0)
        started.extend(wr_c(0, SWITCH, SEM_C))
        issue(wr_c(SWITCH, B - SWITCH, SEM_C + 1))

        r3 = jnp.swapaxes(r_all[...], 0, 1)
        dq_abs = r3[:H] * scale
        ctx_lat = r3[H:]
        ctx_b = _dot(ctx_lat.astype(BF), wuv3[...], BNN).astype(BF)
        dq_b = _dot(dq_abs.astype(BF), wuk3[...], BNN).astype(BF)
        out_att = jnp.sum(_dot(ctx_b, wo[...].reshape(H, D, M), BNN), axis=0)
        dxn = jnp.sum(_dot(dq_b, wq3[...], BNT), axis=0) + dxn_ffn

        os_[...] = (x + out_att + out_ffn).astype(BF)
        dxs[...] = (g + rstd * (dxn - jnp.mean(dxn, axis=-1, keepdims=True)
                                - xn * jnp.mean(dxn * xn, axis=-1, keepdims=True))).astype(BF)
        issue([lambda: pltpu.make_async_copy(os_, o_hbm, wsem.at[SEM_SMALL]),
               lambda: pltpu.make_async_copy(dxs, dx_hbm, wsem.at[SEM_SMALL + 1])])

        n_f = len(ffn_writes)
        ffn_parts = [ffn_writes[k * n_f // 4:(k + 1) * n_f // 4] for k in range(4)]

        wo[...] = _dot(ctx_b, g_bb, BTN).astype(BF).reshape(wo.shape)
        issue(wr_w(wo, dwo_hbm, SEM_W), ffn_parts[0])

        row = jax.lax.broadcasted_iota(jnp.int32, (hh, lanes), 0)
        col = jax.lax.broadcasted_iota(jnp.int32, (hh, lanes), 1)
        own_head = col // B == row
        strips = N_STRIPS // 2

        def weight_grad(y, dst):
            per_run = dst.shape[2]
            cc = strips * per_run

            def body(k, carry):
                r0 = pl.multiple_of(k * cc, cc)
                j0 = (k % 2) * strips
                for t in range(H // hh):
                    xt = xt_ref[pl.ds(r0, cc), t * lanes:(t + 1) * lanes]
                    lhs = jnp.where(own_head[None], xt[:, None, :], 0.0).reshape(cc * hh, lanes).astype(BF)
                    res = _dot(lhs, y[t * lanes:(t + 1) * lanes], NN)
                    dst[k // 2, pl.ds(j0, strips), :, t * hh:(t + 1) * hh, :] = (
                        res.astype(BF).reshape(strips, per_run, hh, D))
                return carry
            jax.lax.fori_loop(0, 2 * dst.shape[0], body, 0)

        xt_ref[...] = ctx_lat.reshape(H * B, CD).T
        weight_grad(dctx_b.reshape(H * B, D), wuv_r)
        xt_ref[...] = dq_abs.reshape(H * B, CD).T
        weight_grad(q_b.reshape(H * B, D), wuk_r)
        xt_ref[...] = jnp.tile(xn.T, (1, H))
        weight_grad(dq_b.reshape(H * B, D), wq_r)

        issue(wr_w(wuv_r, dwuv_hbm, SEM_W + 1), ffn_parts[1])
        issue(wr_w(wuk_r, dwuk_hbm, SEM_W + 2), ffn_parts[2])
        issue(wr_w(wq_r, dwq_hbm, SEM_W + 3), ffn_parts[3])

        for make in started:
            make().wait()

    return kernel


@jax.jit
def pallas_parallel_sum__compressed_kv_cla__geglu_ffn__decode_kernel(
    A_x: jax.Array,
    A_c_kv: jax.Array,
    A_w_q: jax.Array,
    A_w_uk: jax.Array,
    A_w_uv: jax.Array,
    A_w_o: jax.Array,
    B_x: jax.Array,
    B_w_gate: jax.Array,
    B_w_up: jax.Array,
    B_w_down: jax.Array,
    grad_out: jax.Array,
):
    del B_x
    B, SK, CD = A_c_kv.shape
    M, H, D = A_w_q.shape
    F = B_w_gate.shape[1]
    assert M == CD

    def strips(a, run_shape):
        return a.reshape((-1, N_STRIPS) + run_shape)

    x2 = A_x.reshape(B, M)
    g2 = grad_out.reshape(B, M)
    wg_t = B_w_gate.T
    wu_t = B_w_up.T
    c5 = A_c_kv.reshape(B, -1, N_STRIPS, RUN_BYTES // (2 * CD), CD)
    wq5, wuk5, wuv5 = (strips(w, (RUN_BYTES // (2 * H * D), H, D)) for w in (A_w_q, A_w_uk, A_w_uv))
    wo4 = strips(A_w_o, (RUN_BYTES // (2 * M), M))

    def like(a):
        return jax.ShapeDtypeStruct(a.shape, a.dtype)

    vmem = pltpu.VMEM
    scratch = [
        vmem((B, M), BF), vmem((B, M), BF), vmem((B, M), BF), vmem((B, M), BF),
        vmem(c5.shape, BF),
        vmem(wq5.shape, BF), vmem(wuk5.shape, BF), vmem(wuv5.shape, BF),
        vmem(wo4.shape, BF),
        vmem((H, M, D), BF), vmem((H, CD, D), BF), vmem((H, CD, D), BF),
        vmem((F, M), BF), vmem((F, M), BF), vmem((F, M), BF),
        vmem((B, 2 * H, CD), BF), vmem((B, 2 * H, CD), F32),
        vmem((CD, H * B), F32),
        pltpu.SemaphoreType.DMA((11 + B,)), pltpu.SemaphoreType.DMA((11,)),
    ]
    in_hbm = pl.BlockSpec(memory_space=pl.ANY)
    o, dx, dc, dwq, dwuk, dwuv, dwo, dwg_t, dwu_t, dwd = pl.pallas_call(
        _make_kernel(B, SK, CD, M, H, D, F),
        out_shape=[like(x2), like(x2), like(c5), like(wq5), like(wuk5), like(wuv5),
                   like(wo4), like(wg_t), like(wu_t), like(B_w_down)],
        in_specs=[in_hbm] * 10,
        out_specs=[in_hbm] * 10,
        scratch_shapes=scratch,
        compiler_params=pltpu.CompilerParams(vmem_limit_bytes=VMEM_LIMIT,
                                             disable_semaphore_checks=True),
    )(x2, c5, wq5, wuk5, wuv5, wo4, wg_t, wu_t, B_w_down, g2)
    return (o.reshape(A_x.shape), dx.reshape(A_x.shape), dc.reshape(A_c_kv.shape),
            dwq.reshape(A_w_q.shape), dwuk.reshape(A_w_uk.shape), dwuv.reshape(A_w_uv.shape),
            dwo.reshape(A_w_o.shape), dwg_t.T, dwu_t.T, dwd)
```

```python
import jax
import jax.numpy as jnp
from jax.experimental import pallas as pl
from jax.experimental.pallas import tpu as pltpu

BF = jnp.bfloat16
F32 = jnp.float32

NN = (((1,), (0,)), ((), ()))
NT = (((1,), (1,)), ((), ()))
TN = (((0,), (0,)), ((), ()))
BNN = (((2,), (1,)), ((0,), (0,)))
BNT = (((2,), (2,)), ((0,), (0,)))
BTN = (((1,), (1,)), ((0,), (0,)))

LN_EPS = 1e-5
GELU_K0 = 0.7978845608028654
GELU_K1 = 0.044715

RUN_BYTES = 32 * 1024
N_STRIPS = 32
FFN_ROWS = 64
SWITCH = 5
TAIL_STRIPS = 16
VMEM_LIMIT = 110 * 1024 * 1024


def _dot(a, b, dims):
    return jax.lax.dot_general(a, b, dims, preferred_element_type=F32)


def _make_kernel(B, SK, CD, M, H, D, F):
    scale = float(D) ** -0.5
    lanes = 128
    hh = lanes // B
    assert hh * B == lanes and H % hh == 0 and D == lanes
    assert 0 < SWITCH < B - 1

    def kernel(x_hbm, c_hbm, wq_hbm, wuk_hbm, wuv_hbm, wo_hbm, wg_hbm, wu_hbm, wd_hbm, g_hbm,
               o_hbm, dx_hbm, dc_hbm, dwq_hbm, dwuk_hbm, dwuv_hbm, dwo_hbm, dwg_hbm, dwu_hbm, dwd_hbm,
               xs, gs, os_, dxs, cbuf, wq_r, wuk_r, wuv_r, wo, wq3, wuk3, wuv3, wg, wu, wd,
               a_all, r_all, xt_ref, rsem, wsem):
        reads = [(x_hbm, xs), (g_hbm, gs), (wg_hbm, wg), (wu_hbm, wu), (wd_hbm, wd),
                 (wq_hbm, wq_r), (wuk_hbm, wuk_r), (wo_hbm, wo), (wuv_hbm, wuv_r)]
        n_rd = len(reads)
        n_g = cbuf.shape[1]
        keep = N_STRIPS - TAIL_STRIPS

        def rd(i):
            src, dst = reads[i]
            return pltpu.make_async_copy(src, dst, rsem.at[i])

        def rd_c(b):
            return pltpu.make_async_copy(c_hbm.at[b], cbuf.at[b], rsem.at[n_rd + b])

        def rd_last(part):
            idx = [(pl.ds(0, n_g - 1),),
                   (n_g - 1, pl.ds(0, keep)),
                   (n_g - 1, pl.ds(keep, TAIL_STRIPS))][part]
            return pltpu.make_async_copy(c_hbm.at[(B - 1,) + idx], cbuf.at[(B - 1,) + idx],
                                         rsem.at[n_rd + B - 1 + part])

        for i in range(n_rd):
            rd(i).start()
        for b in range(B - 1):
            rd_c(b).start()
        for part in range(3):
            rd_last(part).start()

        def wr_c(b0, nb, sem):
            return [lambda j=j: pltpu.make_async_copy(cbuf.at[pl.ds(b0, nb), :, j],
                                                      dc_hbm.at[pl.ds(b0, nb), :, j], wsem.at[sem])
                    for j in range(N_STRIPS)]

        def wr_w(src, dst, sem):
            return [lambda j=j: pltpu.make_async_copy(src.at[:, j], dst.at[:, j], wsem.at[sem])
                    for j in range(N_STRIPS)]

        ffn = [(wg, dwg_hbm), (wu, dwu_hbm), (wd, dwd_hbm)]
        ffn_writes = []
        for r0 in range(0, F, FFN_ROWS):
            rows = pl.ds(r0, min(FFN_ROWS, F - r0))
            for sem, (src, dst) in enumerate(ffn):
                ffn_writes.append(lambda src=src, dst=dst, rows=rows, sem=sem:
                                  pltpu.make_async_copy(src.at[rows], dst.at[rows], wsem.at[sem]))
        SEM_SMALL, SEM_C, SEM_W = 3, 5, 7

        def issue(copies, extra=()):
            done = 0
            for i, make in enumerate(copies):
                make().start()
                upto = (i + 1) * len(extra) // len(copies)
                for e in extra[done:upto]:
                    e().start()
                done = upto

        rd(0).wait()
        rd(1).wait()
        x = xs[...].astype(F32)
        g_b = gs[...]
        g = g_b.astype(F32)
        xc = x - jnp.mean(x, axis=-1, keepdims=True)
        rstd = jax.lax.rsqrt(jnp.mean(xc * xc, axis=-1, keepdims=True) + LN_EPS)
        xn = xc * rstd
        xn_b = xn.astype(BF)

        rd(2).wait()
        rd(3).wait()
        gate = _dot(xn_b, wg[...], NT)
        up = _dot(xn_b, wu[...], NT)
        th = jnp.tanh(GELU_K0 * (gate + GELU_K1 * gate * gate * gate))
        gl = 0.5 * gate * (1.0 + th)
        dgl = (0.5 * (1.0 + th)
               + 0.5 * gate * (1.0 - th * th) * GELU_K0 * (1.0 + 3.0 * GELU_K1 * gate * gate))
        hid_b = (gl * up).astype(BF)
        rd(4).wait()
        out_ffn = _dot(hid_b, wd[...], NN)
        dh = _dot(g_b, wd[...], NT)
        dgate_b = (dh * up * dgl).astype(BF)
        dup_b = (dh * gl).astype(BF)
        dxn_ffn = _dot(dgate_b, wg[...], NN) + _dot(dup_b, wu[...], NN)
        wg[...] = _dot(dgate_b, xn_b, TN).astype(BF)
        wu[...] = _dot(dup_b, xn_b, TN).astype(BF)
        wd[...] = _dot(hid_b, g_b, TN).astype(BF)

        def head_major(src, dst):
            rows = src.shape[1] * src.shape[2]

            def body(k, carry):
                r0 = pl.multiple_of(k * rows, rows)
                dst[:, pl.ds(r0, rows), :] = jnp.swapaxes(src[k].reshape(rows, H, D), 0, 1)
                return carry
            jax.lax.fori_loop(0, src.shape[0], body, 0)

        rd(5).wait()
        head_major(wq_r, wq3)
        q_b = _dot(jnp.broadcast_to(xn_b[None], (H, B, M)), wq3[...], BNN).astype(BF)
        rd(6).wait()
        head_major(wuk_r, wuk3)
        q_abs = _dot(q_b, wuk3[...], BNT) * scale
        rd(7).wait()
        g_bb = jnp.broadcast_to(g_b[None], (H, B, M))
        dctx_b = _dot(g_bb, wo[...].reshape(H, D, M), BNT).astype(BF)
        rd(8).wait()
        head_major(wuv_r, wuv3)
        dctx_abs = _dot(dctx_b, wuv3[...], BNT)
        a_all[...] = jnp.swapaxes(jnp.concatenate([q_abs, dctx_abs], axis=0), 0, 1).astype(BF)

        def batch(b, carry):
            @pl.when(b < B - 1)
            def _():
                rd_c(b).wait()

            @pl.when(b == B - 1)
            def _():
                rd_last(0).wait()
                rd_last(2).wait()

            @pl.when(b == SWITCH)
            def _():
                rd_last(1).wait()
                issue(wr_c(0, SWITCH, SEM_C))

            a = a_all[b]
            s_all = _dot(a, cbuf[b].reshape(SK, CD), NT)
            s, dp = s_all[:H], s_all[H:]
            e = jnp.exp(s - jnp.max(s, axis=-1, keepdims=True))
            p = e * (1.0 / jnp.sum(e, axis=-1, keepdims=True))
            ds = p * (dp - jnp.sum(p * dp, axis=-1, keepdims=True))
            pm = jnp.concatenate([ds.astype(BF), p.astype(BF)], axis=0)
            r_all[b] = _dot(pm, cbuf[b].reshape(SK, CD), NN)
            cbuf[b] = _dot(pm, a, TN).astype(BF).reshape(cbuf.shape[1:])
            return carry

        jax.lax.fori_loop(0, B, batch, 0)
        issue(wr_c(SWITCH, B - SWITCH, SEM_C + 1))

        r3 = jnp.swapaxes(r_all[...], 0, 1)
        dq_abs = r3[:H] * scale
        ctx_lat = r3[H:]
        ctx_b = _dot(ctx_lat.astype(BF), wuv3[...], BNN).astype(BF)
        dq_b = _dot(dq_abs.astype(BF), wuk3[...], BNN).astype(BF)
        out_att = jnp.sum(_dot(ctx_b, wo[...].reshape(H, D, M), BNN), axis=0)
        dxn = jnp.sum(_dot(dq_b, wq3[...], BNT), axis=0) + dxn_ffn

        os_[...] = (x + out_att + out_ffn).astype(BF)
        dxs[...] = (g + rstd * (dxn - jnp.mean(dxn, axis=-1, keepdims=True)
                                - xn * jnp.mean(dxn * xn, axis=-1, keepdims=True))).astype(BF)
        issue([lambda: pltpu.make_async_copy(os_, o_hbm, wsem.at[SEM_SMALL]),
               lambda: pltpu.make_async_copy(dxs, dx_hbm, wsem.at[SEM_SMALL + 1])])

        wo[...] = _dot(ctx_b, g_bb, BTN).astype(BF).reshape(wo.shape)
        issue(wr_w(wo, dwo_hbm, SEM_W))

        row = jax.lax.broadcasted_iota(jnp.int32, (hh, lanes), 0)
        col = jax.lax.broadcasted_iota(jnp.int32, (hh, lanes), 1)
        own_head = col // B == row
        strips = N_STRIPS // 2

        def weight_grad(y, dst):
            per_run = dst.shape[2]
            cc = strips * per_run

            def body(k, carry):
                r0 = pl.multiple_of(k * cc, cc)
                j0 = (k % 2) * strips
                for t in range(H // hh):
                    xt = xt_ref[pl.ds(r0, cc), t * lanes:(t + 1) * lanes]
                    lhs = jnp.where(own_head[None], xt[:, None, :], 0.0).reshape(cc * hh, lanes).astype(BF)
                    res = _dot(lhs, y[t * lanes:(t + 1) * lanes], NN)
                    dst[k // 2, pl.ds(j0, strips), :, t * hh:(t + 1) * hh, :] = (
                        res.astype(BF).reshape(strips, per_run, hh, D))
                return carry
            jax.lax.fori_loop(0, 2 * dst.shape[0], body, 0)

        xt_ref[...] = ctx_lat.reshape(H * B, CD).T
        weight_grad(dctx_b.reshape(H * B, D), wuv_r)
        xt_ref[...] = dq_abs.reshape(H * B, CD).T
        weight_grad(q_b.reshape(H * B, D), wuk_r)
        xt_ref[...] = jnp.tile(xn.T, (1, H))
        weight_grad(dq_b.reshape(H * B, D), wq_r)

        n_f = len(ffn_writes)
        last = [(wuv_r, dwuv_hbm), (wuk_r, dwuk_hbm), (wq_r, dwq_hbm)]
        for k, (src, dst) in enumerate(last):
            issue(wr_w(src, dst, SEM_W + 1 + k), ffn_writes[k * n_f // 3:(k + 1) * n_f // 3])

        first, rest = pl.ds(0, SWITCH), pl.ds(SWITCH, B - SWITCH)
        totals = [(cbuf.at[first], dc_hbm.at[first], SEM_C), (cbuf.at[rest], dc_hbm.at[rest], SEM_C + 1),
                  (os_, o_hbm, SEM_SMALL), (dxs, dx_hbm, SEM_SMALL + 1), (wo, dwo_hbm, SEM_W)]
        totals += [(src, dst, SEM_W + 1 + k) for k, (src, dst) in enumerate(last)]
        totals += [(src, dst, sem) for sem, (src, dst) in enumerate(ffn)]
        for src, dst, sem in totals:
            pltpu.make_async_copy(src, dst, wsem.at[sem]).wait()

    return kernel


@jax.jit
def pallas_parallel_sum__compressed_kv_cla__geglu_ffn__decode_kernel(
    A_x: jax.Array,
    A_c_kv: jax.Array,
    A_w_q: jax.Array,
    A_w_uk: jax.Array,
    A_w_uv: jax.Array,
    A_w_o: jax.Array,
    B_x: jax.Array,
    B_w_gate: jax.Array,
    B_w_up: jax.Array,
    B_w_down: jax.Array,
    grad_out: jax.Array,
):
    del B_x
    B, SK, CD = A_c_kv.shape
    M, H, D = A_w_q.shape
    F = B_w_gate.shape[1]
    assert M == CD

    def strips(a, run_shape):
        return a.reshape((-1, N_STRIPS) + run_shape)

    x2 = A_x.reshape(B, M)
    g2 = grad_out.reshape(B, M)
    wg_t = B_w_gate.T
    wu_t = B_w_up.T
    c5 = A_c_kv.reshape(B, -1, N_STRIPS, RUN_BYTES // (2 * CD), CD)
    wq5, wuk5, wuv5 = (strips(w, (RUN_BYTES // (2 * H * D), H, D)) for w in (A_w_q, A_w_uk, A_w_uv))
    wo4 = strips(A_w_o, (RUN_BYTES // (2 * M), M))

    def like(a):
        return jax.ShapeDtypeStruct(a.shape, a.dtype)

    vmem = pltpu.VMEM
    scratch = [
        vmem((B, M), BF), vmem((B, M), BF), vmem((B, M), BF), vmem((B, M), BF),
        vmem(c5.shape, BF),
        vmem(wq5.shape, BF), vmem(wuk5.shape, BF), vmem(wuv5.shape, BF),
        vmem(wo4.shape, BF),
        vmem((H, M, D), BF), vmem((H, CD, D), BF), vmem((H, CD, D), BF),
        vmem((F, M), BF), vmem((F, M), BF), vmem((F, M), BF),
        vmem((B, 2 * H, CD), BF), vmem((B, 2 * H, CD), F32),
        vmem((CD, H * B), F32),
        pltpu.SemaphoreType.DMA((11 + B,)), pltpu.SemaphoreType.DMA((11,)),
    ]
    in_hbm = pl.BlockSpec(memory_space=pl.ANY)
    o, dx, dc, dwq, dwuk, dwuv, dwo, dwg_t, dwu_t, dwd = pl.pallas_call(
        _make_kernel(B, SK, CD, M, H, D, F),
        out_shape=[like(x2), like(x2), like(c5), like(wq5), like(wuk5), like(wuv5),
                   like(wo4), like(wg_t), like(wu_t), like(B_w_down)],
        in_specs=[in_hbm] * 10,
        out_specs=[in_hbm] * 10,
        scratch_shapes=scratch,
        compiler_params=pltpu.CompilerParams(vmem_limit_bytes=VMEM_LIMIT,
                                             disable_semaphore_checks=True),
    )(x2, c5, wq5, wuk5, wuv5, wo4, wg_t, wu_t, B_w_down, g2)
    return (o.reshape(A_x.shape), dx.reshape(A_x.shape), dc.reshape(A_c_kv.shape),
            dwq.reshape(A_w_q.shape), dwuk.reshape(A_w_uk.shape), dwuv.reshape(A_w_uv.shape),
            dwo.reshape(A_w_o.shape), dwg_t.T, dwu_t.T, dwd)
```
